```python
import jax
import jax.numpy as jnp

def _softmax(x, axis=-1):
    return jax.nn.softmax(x, axis=axis)
def _gelu(x):
    return jax.nn.gelu(x, approximate=True)
def _silu(x):
    return jax.nn.silu(x)
def _sigmoid(x):
    return jax.nn.sigmoid(x)
def _layernorm(x, axis=-1, eps=1e-5):
    m = jnp.mean(x, axis=axis, keepdims=True)
    v = jnp.var(x, axis=axis, keepdims=True)
    return (x - m) / jnp.sqrt(v + eps)
def _scatter_add(tgt, idx, src, axis=0):
    return tgt.at[idx].add(src)
def _segment_sum(src, seg, n):
    return jax.ops.segment_sum(src, seg, n)
class _Rng:
    def __init__(self, key):
        self._k = key
    def _next(self):
        self._k, sub = jax.random.split(self._k)
        return sub
    def normal(self, shape):
        return jax.random.normal(self._next(), shape, dtype=jnp.bfloat16)
    def randint(self, lo, hi, shape):
        return jax.random.randint(self._next(), shape, lo, hi, dtype=jnp.int32)
    def uniform(self, shape, lo=0.0, hi=1.0):
        return jax.random.uniform(self._next(), shape, jnp.bfloat16, lo, hi)
    def permutation(self, n):
        return jax.random.permutation(self._next(), n)


kernel_name = 'recurrent_scan__compressed_kv_cla__dense_activation_silu__decode'

def setup_inputs():
    _rng = _Rng(jax.random.key(int.from_bytes(__import__("os").urandom(4), "little")))
    _w = (lambda a: (lambda t: t.astype(jnp.bfloat16) if jnp.issubdtype(t.dtype, jnp.floating) else t)(jnp.asarray(a)))
    def _A_setup():
        B, H, Sq, Sk, D, M = 1, 32, 1, 32768, 128, 512
        Dc = 4 * D
        return {
            "x": _w((lambda *s: _rng.normal(s) * 0.05)(B, Sq, M)),
            "c_kv": _w((lambda *s: _rng.normal(s) * 0.05)(B, Sk, Dc)),
            "w_q": _w((lambda *s: _rng.normal(s) * 0.05)(M, H, D) * (M ** -0.5)),
            "w_uk": _w((lambda *s: _rng.normal(s) * 0.05)(Dc, H, D) * (Dc ** -0.5)),
            "w_uv": _w((lambda *s: _rng.normal(s) * 0.05)(Dc, H, D) * (Dc ** -0.5)),
            "w_o": _w((lambda *s: _rng.normal(s) * 0.05)(H, D, M) * ((H * D) ** -0.5)),
        }
    _A_in = _A_setup()

    def _B_setup():
        B, S, D, F = 1, 1, 512, 1376
        return {
            "x": _w((lambda *s: _rng.normal(s) * 0.05)(B, S, D)),
            "w1": _w((lambda *s: _rng.normal(s) * 0.05)(D, F) * (D ** -0.5)),
            "w2": _w((lambda *s: _rng.normal(s) * 0.05)(F, D) * (F ** -0.5)),
        }
    _B_in = _B_setup()

    return {
        "A_x": _A_in["x"],
        "A_c_kv": _A_in["c_kv"],
        "A_w_q": _A_in["w_q"],
        "A_w_uk": _A_in["w_uk"],
        "A_w_uv": _A_in["w_uv"],
        "A_w_o": _A_in["w_o"],
        "B_x": _B_in["x"],
        "B_w1": _B_in["w1"],
        "B_w2": _B_in["w2"],
    }

def reference(A_x, A_c_kv, A_w_q, A_w_uk, A_w_uv, A_w_o, B_x, B_w1, B_w2):
    def _A_ref(x, c_kv, w_q, w_uk, w_uv, w_o):
        B, Sq, M = x.shape[0], x.shape[1], x.shape[2]
        Sk = c_kv.shape[1]
        H, D = w_q.shape[1], w_q.shape[2]
        q = jnp.einsum("bqm,mhd->bhqd", x, w_q)
        k = jnp.einsum("bkc,chd->bhkd", c_kv, w_uk)
        v = jnp.einsum("bkc,chd->bhkd", c_kv, w_uv)
        scores = jnp.einsum("bhqd,bhkd->bhqk", q, k) * (D ** -0.5)
        off = Sk - Sq
        qi = jnp.arange(Sq)[:, None]
        kj = jnp.arange(Sk)[None, :]
        cmask = kj <= (qi + off)
        scores = jnp.where(cmask[None, None], scores, -1e9)
        p = _softmax(scores, axis=-1)
        ctx = jnp.einsum("bhqk,bhkd->bhqd", p, v)
        return jnp.einsum("bhqd,hdm->bqm", ctx, w_o)

    def _B_ref(x, w1, w2):
        h = jnp.einsum("bsd,df->bsf", x, w1)
        h = _silu(h)
        out = jnp.einsum("bsf,fd->bsd", h, w2)
        return out

    x = A_x
    xn = _layernorm(x, axis=-1)
    s = _A_ref(xn, A_c_kv, A_w_q, A_w_uk, A_w_uv, A_w_o)
    g = _silu(_B_ref(xn, B_w1, B_w2))
    return x + s * g
```

```python
import functools
import jax
import jax.numpy as jnp
import numpy as np
from jax import lax
from jax.experimental import pallas as pl
from jax.experimental.pallas import tpu as pltpu

H, D, M, DC, SK, F = 32, 128, 512, 512, 32768, 1376
LOG2E = 1.4426950408889634


def _make(chunk=4096, bk=1024, wo_last=4):
    nchunk = SK // chunk
    nb_chunk = chunk // bk

    def kernel(x_hbm, ckv_hbm, wq_hbm, wuk_hbm, wuv_hbm, wo_hbm, w1_hbm, w2_hbm, o_ref,
               x_v, ckv_v, wq_v, wuk_v, wuv_v, wo_v, w1_v, w2_v, qabs_v, ctxc_v, sems):
        cp_wq = pltpu.make_async_copy(wq_hbm, wq_v, sems.at[0])
        cp_x = pltpu.make_async_copy(x_hbm.at[0], x_v, sems.at[1])
        cp_wuk = pltpu.make_async_copy(wuk_hbm, wuk_v, sems.at[2])
        cp_w1 = pltpu.make_async_copy(w1_hbm, w1_v, sems.at[3])
        cp_w2 = pltpu.make_async_copy(w2_hbm, w2_v, sems.at[4])
        cp_wuv = pltpu.make_async_copy(wuv_hbm, wuv_v, sems.at[5])
        h0 = H - wo_last
        cp_wo0 = pltpu.make_async_copy(wo_hbm.at[pl.ds(0, h0)], wo_v.at[pl.ds(0, h0)], sems.at[6])
        cp_wo1 = pltpu.make_async_copy(wo_hbm.at[pl.ds(h0, wo_last)], wo_v.at[pl.ds(h0, wo_last)], sems.at[7])

        def cp_ckv(j):
            return pltpu.make_async_copy(ckv_hbm.at[0, pl.ds(j * chunk, chunk), :],
                                         ckv_v.at[pl.ds(j * chunk, chunk), :], sems.at[8 + j])

        cp_wq.start()
        cp_x.start()
        cp_wuk.start()
        for j in range(nchunk):
            cp_ckv(j).start()
        cp_wuv.start()
        cp_w1.start()
        cp_w2.start()
        cp_wo0.start()
        cp_wo1.start()

        lane = lax.broadcasted_iota(jnp.int32, (H, 128), 1)
        row = lax.broadcasted_iota(jnp.int32, (H, 128), 0)
        diag = (lane & 31) == row
        grp = lane >> 5

        def expand(v_tile):
            outs = []
            for t in range(32):
                a = jnp.take_along_axis(v_tile, grp + 4 * t, axis=1)
                outs.append(jnp.where(diag, a, 0.0).astype(jnp.bfloat16))
            return jnp.concatenate(outs, axis=1)

        cp_x.wait()
        x = x_v[...].astype(jnp.float32)
        mean = jnp.sum(x, axis=1, keepdims=True) * (1.0 / M)
        xc = x - mean
        var = jnp.sum(xc * xc, axis=1, keepdims=True) * (1.0 / M)
        xn = xc * lax.rsqrt(var + 1e-5)
        xb = jnp.broadcast_to(xn, (H, M))

        cp_wq.wait()
        q = jnp.zeros((H, D), jnp.float32)
        for i in range(M // 128):
            a = expand(xb[:, 128 * i:128 * (i + 1)])
            w = wq_v[128 * i:128 * (i + 1)].reshape(128 * H, D)
            q = q + jnp.dot(a, w, preferred_element_type=jnp.float32)
        qb = q.astype(jnp.bfloat16)

        cp_wuk.wait()
        idx_c = 32 * (lane & 3) + row
        lane4 = lane >> 2
        for i in range(DC // 128):
            w = wuk_v[128 * i:128 * (i + 1)].reshape(128 * H, D)
            T = lax.dot_general(qb, w, (((1,), (1,)), ((), ())), preferred_element_type=jnp.float32)
            out = jnp.zeros((H, 128), jnp.float32)
            for t in range(32):
                G = jnp.take_along_axis(T[:, 128 * t:128 * (t + 1)], idx_c, axis=1)
                out = jnp.where(lane4 == t, G, out)
            qabs_v[:, 128 * i:128 * (i + 1)] = (out * (D ** -0.5 * LOG2E)).astype(jnp.bfloat16)
        qa = qabs_v[...]

        def blk(b, carry):
            m, l, acc = carry
            c = ckv_v[pl.ds(pl.multiple_of(b * bk, bk), bk), :]
            s = lax.dot_general(qa, c, (((1,), (1,)), ((), ())), preferred_element_type=jnp.float32)
            m_new = jnp.maximum(m, jnp.max(s, axis=1, keepdims=True))
            alpha = jnp.exp2(m - m_new)
            p = jnp.exp2(s - m_new)
            l = alpha * l + jnp.sum(p, axis=1, keepdims=True)
            acc = alpha * acc + jnp.dot(p.astype(jnp.bfloat16), c, preferred_element_type=jnp.float32)
            return m_new, l, acc

        carry = (jnp.full((H, 1), -jnp.inf, jnp.float32), jnp.zeros((H, 1), jnp.float32),
                 jnp.zeros((H, DC), jnp.float32))
        for j in range(nchunk):
            cp_ckv(j).wait()
            carry = lax.fori_loop(j * nb_chunk, (j + 1) * nb_chunk, blk, carry)
        m, l, acc = carry
        ctxc = acc / l

        cp_wuv.wait()
        ctx = jnp.zeros((H, D), jnp.float32)
        for i in range(DC // 128):
            a = expand(ctxc[:, 128 * i:128 * (i + 1)])
            w = wuv_v[128 * i:128 * (i + 1)].reshape(128 * H, D)
            ctx = ctx + jnp.dot(a, w, preferred_element_type=jnp.float32)

        cp_w1.wait()
        xb16 = jnp.broadcast_to(xn, (16, M)).astype(jnp.bfloat16)
        h1 = lax.dot_general(xb16, w1_v[...], (((1,), (1,)), ((), ())), preferred_element_type=jnp.float32)
        h1 = h1 * jax.nn.sigmoid(h1)
        cp_w2.wait()
        g = jnp.dot(h1.astype(jnp.bfloat16), w2_v[...], preferred_element_type=jnp.float32)
        g = g[0:1]
        g = g * jax.nn.sigmoid(g)

        def a_o(hs):
            return jnp.concatenate(
                [jnp.where(row == h, ctx, 0.0).astype(jnp.bfloat16) for h in hs], axis=1)

        cp_wo0.wait()
        s = jnp.dot(a_o(range(h0)), wo_v[0:h0].reshape(h0 * D, M), preferred_element_type=jnp.float32)
        a1 = a_o(range(h0, H))
        cp_wo1.wait()
        s = s + jnp.dot(a1, wo_v[h0:H].reshape(wo_last * D, M), preferred_element_type=jnp.float32)
        s = jnp.sum(s, axis=0, keepdims=True)
        o_ref[0] = (x + s * g).astype(o_ref.dtype)

    def f(A_x, A_c_kv, A_w_q, A_w_uk, A_w_uv, A_w_o, B_x, B_w1, B_w2):
        any_spec = pl.BlockSpec(memory_space=pl.ANY)
        return pl.pallas_call(
            kernel,
            in_specs=[any_spec] * 8,
            out_specs=pl.BlockSpec(memory_space=pltpu.VMEM),
            out_shape=jax.ShapeDtypeStruct((1, 1, M), jnp.bfloat16),
            scratch_shapes=[
                pltpu.VMEM((1, M), jnp.bfloat16),
                pltpu.VMEM((SK, DC), jnp.bfloat16),
                pltpu.VMEM((M, H, D), jnp.bfloat16),
                pltpu.VMEM((DC, H, D), jnp.bfloat16),
                pltpu.VMEM((DC, H, D), jnp.bfloat16),
                pltpu.VMEM((H, D, M), jnp.bfloat16),
                pltpu.VMEM((F, M), jnp.bfloat16),
                pltpu.VMEM((F, M), jnp.bfloat16),
                pltpu.VMEM((H, DC), jnp.bfloat16),
                pltpu.VMEM((H, DC), jnp.float32),
                pltpu.SemaphoreType.DMA((8 + nchunk,)),
            ],
            compiler_params=pltpu.CompilerParams(vmem_limit_bytes=100 * 1024 * 1024),
        )(A_x, A_c_kv, A_w_q, A_w_uk, A_w_uv, A_w_o, B_w1.T, B_w2)
    return f


_KERNEL = _make()


@jax.jit
def pallas_recurrent_scan__compressed_kv_cla__dense_activation_silu__decode_kernel(
    A_x: jax.Array,
    A_c_kv: jax.Array,
    A_w_q: jax.Array,
    A_w_uk: jax.Array,
    A_w_uv: jax.Array,
    A_w_o: jax.Array,
    B_x: jax.Array,
    B_w1: jax.Array,
    B_w2: jax.Array,
):
    return _KERNEL(A_x, A_c_kv, A_w_q, A_w_uk, A_w_uv, A_w_o, B_x, B_w1, B_w2)
```

```python
import jax
import jax.numpy as jnp
from jax import lax
import jax.experimental.pallas as pl
import jax.experimental.pallas.tpu as pltpu

_LOG2E = 1.4426950408889634
_LN_EPS = 1e-5

_N_KV_CHUNKS = 4
_KV_BLOCK = 1024
_WO_MXU_HEADS = (24, 4, 2)
_WO_VPU_ROWS = (128, 96, 16, 16)


def _kernel_body(H, D, M, DC, SK, HV,
                 x_hbm, ckv_hbm, wq_hbm, wuk_hbm, wuv_hbm, wo_hbm, w1t_hbm, w2_hbm, o_hbm,
                 x_v, ckv_v, wq_v, wuk_v, wuv_v, wo_v, w1t_v, w2_v,
                 xn_v, xt_v, q_v, qb_v, qabs_v, ctxc_v, ctx_v, h1_v, g_v, s_v, cw_v,
                 base_v, acc_v, o_v):
    f32, bf16 = jnp.float32, jnp.bfloat16
    n_ck = _N_KV_CHUNKS
    chunk = SK // n_ck
    blocks_per_chunk = chunk // _KV_BLOCK
    n_m, n_v = len(_WO_MXU_HEADS), len(_WO_VPU_ROWS)
    h_off = [sum(_WO_MXU_HEADS[:j]) for j in range(n_m + 1)]
    r_off = [sum(_WO_VPU_ROWS[:j]) for j in range(n_v + 1)]
    HM = h_off[-1]
    n_sem = 7 + n_ck + n_m + n_v
    GRP = 128 // H
    TPB = H

    def iotas():
        return (lax.broadcasted_iota(jnp.int32, (H, 128), 1),
                lax.broadcasted_iota(jnp.int32, (H, 128), 0))

    def block_diag(v):
        lane, row = iotas()
        diag = (lane % H) == row
        grp = lane // H
        tiles = []
        for t in range(TPB):
            a = jnp.take_along_axis(v, grp + GRP * t, axis=1)
            tiles.append(jnp.where(diag, a, 0.0).astype(bf16))
        return jnp.concatenate(tiles, axis=1)

    def head_matvec(v_ref, w_ref, out_ref, n_blocks):
        out_ref[...] = jnp.zeros((H, D), f32)

        def body(i, _):
            a = block_diag(v_ref[i])
            w = w_ref[pl.ds(pl.multiple_of(i * 128, 128), 128)].reshape(128 * H, D)
            out_ref[...] += jnp.dot(a, w, preferred_element_type=f32)

        lax.fori_loop(0, n_blocks, body, None)

    def scoped(S):
        cp_wq = pltpu.make_async_copy(wq_hbm, wq_v, S.at[0])
        cp_x = pltpu.make_async_copy(x_hbm.at[0], x_v, S.at[1])
        cp_wuk = pltpu.make_async_copy(wuk_hbm, wuk_v, S.at[2])
        cp_wuv = pltpu.make_async_copy(wuv_hbm, wuv_v, S.at[3])
        cp_w1 = pltpu.make_async_copy(w1t_hbm, w1t_v, S.at[4])
        cp_w2 = pltpu.make_async_copy(w2_hbm, w2_v, S.at[5])
        cp_out = pltpu.make_async_copy(o_v, o_hbm.at[0], S.at[6])

        def cp_ckv(j):
            sl = pl.ds(j * chunk, chunk)
            return pltpu.make_async_copy(ckv_hbm.at[0, sl, :], ckv_v.at[sl, :], S.at[7 + j])

        def cp_wo_mxu(j):
            sl = pl.ds(h_off[j], _WO_MXU_HEADS[j])
            return pltpu.make_async_copy(wo_hbm.at[sl], wo_v.at[sl], S.at[7 + n_ck + j])

        def cp_wo_vpu(j):
            h = HM + r_off[j] // D
            sl = pl.ds(r_off[j] % D, _WO_VPU_ROWS[j])
            return pltpu.make_async_copy(wo_hbm.at[h, sl, :], wo_v.at[h, sl, :],
                                         S.at[7 + n_ck + n_m + j])

        cp_wq.start()
        cp_x.start()
        cp_wuk.start()
        for j in range(n_ck):
            cp_ckv(j).start()
        cp_wuv.start()
        cp_w1.start()
        cp_w2.start()
        for j in range(n_m):
            cp_wo_mxu(j).start()
        for j in range(n_v):
            cp_wo_vpu(j).start()

        cp_x.wait()
        x = x_v[...].astype(f32)
        mean = jnp.sum(x, axis=1, keepdims=True) * (1.0 / M)
        xc = x - mean
        var = jnp.sum(xc * xc, axis=1, keepdims=True) * (1.0 / M)
        xn = xc * lax.rsqrt(var + _LN_EPS)
        xn_v[...] = jnp.broadcast_to(xn, xn_v.shape).astype(bf16)
        for i in range(M // 128):
            xt_v[i] = jnp.broadcast_to(xn[:, 128 * i:128 * (i + 1)], (H, 128))

        cp_wq.wait()
        head_matvec(xt_v, wq_v, q_v, M // 128)
        qb_v[...] = q_v[...].astype(bf16)

        cp_wuk.wait()

        def qabs_body(i, _):
            lane, row = iotas()
            w = wuk_v[pl.ds(pl.multiple_of(i * 128, 128), 128)].reshape(128 * H, D)
            T = lax.dot_general(qb_v[...], w, (((1,), (1,)), ((), ())),
                                preferred_element_type=f32)
            idx = H * (lane % GRP) + row
            sel = lane // GRP
            out = jnp.zeros((H, 128), f32)
            for t in range(TPB):
                g = jnp.take_along_axis(T[:, 128 * t:128 * (t + 1)], idx, axis=1)
                out = jnp.where(sel == t, g, out)
            qabs_v[i] = (out * (D ** -0.5 * _LOG2E)).astype(bf16)

        lax.fori_loop(0, DC // 128, qabs_body, None)

        def kv_block(b, carry):
            m, l, acc = carry
            qa = jnp.concatenate([qabs_v[i] for i in range(DC // 128)], axis=1)
            c = ckv_v[pl.ds(pl.multiple_of(b * _KV_BLOCK, _KV_BLOCK), _KV_BLOCK), :]
            s = lax.dot_general(qa, c, (((1,), (1,)), ((), ())),
                                preferred_element_type=f32)
            m_new = jnp.maximum(m, jnp.max(s, axis=1, keepdims=True))
            alpha = jnp.exp2(m - m_new)
            p = jnp.exp2(s - m_new)
            l = alpha * l + jnp.sum(p, axis=1, keepdims=True)
            acc = alpha * acc + jnp.dot(p.astype(bf16), c, preferred_element_type=f32)
            return m_new, l, acc

        def kv_chunk(j, carry):
            cp_ckv(j).wait()
            return lax.fori_loop(j * blocks_per_chunk, (j + 1) * blocks_per_chunk,
                                 kv_block, carry)

        _, l, acc = lax.fori_loop(
            0, n_ck, kv_chunk,
            (jnp.full((H, 1), -jnp.inf, f32), jnp.zeros((H, 1), f32), jnp.zeros((H, DC), f32)))
        ctxc = acc / l
        for i in range(DC // 128):
            ctxc_v[i] = ctxc[:, 128 * i:128 * (i + 1)]

        cp_wuv.wait()
        head_matvec(ctxc_v, wuv_v, ctx_v, DC // 128)
        for hh in range(HV):
            r = ctx_v[HM + hh:HM + hh + 1, :]
            cw_v[hh * D:(hh + 1) * D, :] = jnp.broadcast_to(r, (128, D)).T

        cp_w1.wait()
        h1 = lax.dot_general(xn_v[...], w1t_v[...], (((1,), (1,)), ((), ())),
                             preferred_element_type=f32)
        h1_v[...] = (h1 * jax.nn.sigmoid(h1)).astype(bf16)
        cp_w2.wait()
        g = jnp.dot(h1_v[...], w2_v[...], preferred_element_type=f32)[0:1]
        g_v[...] = g * jax.nn.sigmoid(g)

        for j in range(n_m):
            h0, h1_ = h_off[j], h_off[j + 1]
            ctx = ctx_v[...]
            _, row = iotas()
            a = jnp.concatenate(
                [jnp.where(row == h, ctx, 0.0).astype(bf16) for h in range(h0, h1_)], axis=1)
            cp_wo_mxu(j).wait()
            sj = jnp.dot(a, wo_v[h0:h1_].reshape((h1_ - h0) * D, M),
                         preferred_element_type=f32)
            if j > 0:
                sj = sj + s_v[...]
            if j < n_m - 1:
                s_v[...] = sj
            else:
                s = jnp.sum(sj, axis=0, keepdims=True)
                base_v[...] = x_v[...].astype(f32) + s * g_v[...]

        for j in range(n_v):
            h = HM + r_off[j] // D
            r0, R = r_off[j] % D, _WO_VPU_ROWS[j]
            c = cw_v[r_off[j]:r_off[j] + R, :]
            cp_wo_vpu(j).wait()
            w = wo_v[h, r0:r0 + R, :].astype(f32)
            p = w * jnp.concatenate([c] * (M // 128), axis=1)
            acc = jnp.sum(p.reshape(R // 8, 8, M), axis=0)
            if j > 0:
                acc = acc + acc_v[...]
            if j < n_v - 1:
                acc_v[...] = acc
            else:
                s = jnp.sum(acc, axis=0, keepdims=True)
                o_v[...] = (base_v[...] + s * g_v[...]).astype(o_v.dtype)

        cp_out.start()
        cp_out.wait()

    pl.run_scoped(scoped, pltpu.SemaphoreType.DMA((n_sem,)))


@jax.jit
def pallas_recurrent_scan__compressed_kv_cla__dense_activation_silu__decode_kernel(
    A_x: jax.Array,
    A_c_kv: jax.Array,
    A_w_q: jax.Array,
    A_w_uk: jax.Array,
    A_w_uv: jax.Array,
    A_w_o: jax.Array,
    B_x: jax.Array,
    B_w1: jax.Array,
    B_w2: jax.Array,
):
    del B_x
    B, Sq, M = A_x.shape
    _, SK, DC = A_c_kv.shape
    _, H, D = A_w_q.shape
    F = B_w1.shape[1]
    assert B == 1 and Sq == 1, "single-token decode"
    assert D == 128 and 128 % H == 0 and M % 128 == 0 and DC % 128 == 0
    assert SK % (_N_KV_CHUNKS * _KV_BLOCK) == 0
    HM = sum(_WO_MXU_HEADS)
    HV = H - HM
    assert sum(_WO_VPU_ROWS) == HV * D

    def kernel(*refs):
        _kernel_body(H, D, M, DC, SK, HV, *refs)

    hbm = pl.BlockSpec(memory_space=pl.ANY)
    f32, bf16 = jnp.float32, jnp.bfloat16
    return pl.pallas_call(
        kernel,
        in_specs=[hbm] * 8,
        out_specs=hbm,
        out_shape=jax.ShapeDtypeStruct((1, 1, M), A_x.dtype),
        scratch_shapes=[
            pltpu.VMEM((1, M), A_x.dtype),
            pltpu.VMEM((SK, DC), A_c_kv.dtype),
            pltpu.VMEM((M, H, D), A_w_q.dtype),
            pltpu.VMEM((DC, H, D), A_w_uk.dtype),
            pltpu.VMEM((DC, H, D), A_w_uv.dtype),
            pltpu.VMEM((H, D, M), A_w_o.dtype),
            pltpu.VMEM((F, M), B_w1.dtype),
            pltpu.VMEM((F, M), B_w2.dtype),
            pltpu.VMEM((16, M), bf16),
            pltpu.VMEM((M // 128, H, 128), f32),
            pltpu.VMEM((H, D), f32),
            pltpu.VMEM((H, D), bf16),
            pltpu.VMEM((DC // 128, H, 128), bf16),
            pltpu.VMEM((DC // 128, H, 128), f32),
            pltpu.VMEM((H, D), f32),
            pltpu.VMEM((16, F), bf16),
            pltpu.VMEM((1, M), f32),
            pltpu.VMEM((H, M), f32),
            pltpu.VMEM((HV * D, 128), f32),
            pltpu.VMEM((1, M), f32),
            pltpu.VMEM((8, M), f32),
            pltpu.VMEM((1, M), A_x.dtype),
        ],
        compiler_params=pltpu.CompilerParams(vmem_limit_bytes=64 * 1024 * 1024),
    )(A_x, A_c_kv, A_w_q, A_w_uk, A_w_uv, A_w_o,
      B_w1.T,
      B_w2)
```

```python
import jax
import jax.numpy as jnp
from jax import lax
import jax.experimental.pallas as pl
import jax.experimental.pallas.tpu as pltpu

_LOG2E = 1.4426950408889634
_LN_EPS = 1e-5

_N_KV_CHUNKS = 8
_KV_BLOCK = 1024
_WO_SIDE_HEADS = _N_KV_CHUNKS + 3
_WO_MXU_HEADS = (24, 4, 2)
_WO_VPU_ROWS = (128, 96, 16, 16)


def _kernel_body(H, D, M, DC, SK, HV,
                 x_hbm, ckv_hbm, wq_hbm, wuk_hbm, wuv_hbm, wo_hbm, w1t_hbm, w2_hbm, o_hbm,
                 x_v, ckv_v, wq_v, wuk_v, wuv_v, wo_v, w1t_v, w2_v,
                 xn_v, xt_v, q_v, qb_v, qabs_v, ctxc_v, ctx_v, h1_v, g_v, s_v, cw_v,
                 base_v, acc_v, o_v, sm):
    f32, bf16 = jnp.float32, jnp.bfloat16
    n_ck = _N_KV_CHUNKS
    chunk = SK // n_ck
    blocks_per_chunk = chunk // _KV_BLOCK
    n_m, n_v = len(_WO_MXU_HEADS), len(_WO_VPU_ROWS)
    h_off = [sum(_WO_MXU_HEADS[:j]) for j in range(n_m + 1)]
    r_off = [sum(_WO_VPU_ROWS[:j]) for j in range(n_v + 1)]
    HM = h_off[-1]
    n_sem = 7 + n_ck + n_m + n_v
    n_side = _WO_SIDE_HEADS
    GRP = 128 // H
    TPB = H

    def iotas():
        return (lax.broadcasted_iota(jnp.int32, (H, 128), 1),
                lax.broadcasted_iota(jnp.int32, (H, 128), 0))

    def block_diag(v):
        lane, row = iotas()
        diag = (lane % H) == row
        grp = lane // H
        tiles = []
        for t in range(TPB):
            a = jnp.take_along_axis(v, grp + GRP * t, axis=1)
            tiles.append(jnp.where(diag, a, 0.0).astype(bf16))
        return jnp.concatenate(tiles, axis=1)

    def head_matvec(v_ref, w_ref, out_ref, n_blocks):
        out_ref[...] = jnp.zeros((H, D), f32)

        def body(i, _):
            a = block_diag(v_ref[i])
            w = w_ref[pl.ds(pl.multiple_of(i * 128, 128), 128)].reshape(128 * H, D)
            out_ref[...] += jnp.dot(a, w, preferred_element_type=f32)

        lax.fori_loop(0, n_blocks, body, None)

    def scoped(S, SI, SO):
        cp_wq = pltpu.make_async_copy(wq_hbm, wq_v, S.at[0])
        cp_x = pltpu.make_async_copy(x_hbm.at[0], x_v, S.at[1])
        cp_wuk = pltpu.make_async_copy(wuk_hbm, wuk_v, S.at[2])
        cp_wuv = pltpu.make_async_copy(wuv_hbm, wuv_v, S.at[3])
        cp_w1 = pltpu.make_async_copy(w1t_hbm, w1t_v, S.at[4])
        cp_w2 = pltpu.make_async_copy(w2_hbm, w2_v, S.at[5])
        cp_out = pltpu.make_async_copy(o_v, o_hbm.at[0], S.at[6])

        def cp_ckv(j):
            sl = pl.ds(j * chunk, chunk)
            return pltpu.make_async_copy(ckv_hbm.at[0, sl, :], ckv_v.at[sl, :], S.at[7 + j])

        def cp_wo_mxu(j):
            lo = max(h_off[j], n_side)
            sl = pl.ds(lo, h_off[j + 1] - lo)
            return pltpu.make_async_copy(wo_hbm.at[sl], wo_v.at[sl], S.at[7 + n_ck + j])

        def cp_in(i):
            return pltpu.make_async_copy(wo_hbm.at[i], sm.at[i % 2], SI.at[i % 2])

        def cp_fwd(i):
            return pltpu.make_async_copy(sm.at[i % 2], wo_v.at[i], SO.at[i % 2])

        def side_tick(i):
            cp_in(i - 1).wait()
            cp_fwd(i - 2).wait()
            cp_fwd(i - 1).start()
            cp_in(i).start()

        def cp_wo_vpu(j):
            h = HM + r_off[j] // D
            sl = pl.ds(r_off[j] % D, _WO_VPU_ROWS[j])
            return pltpu.make_async_copy(wo_hbm.at[h, sl, :], wo_v.at[h, sl, :],
                                         S.at[7 + n_ck + n_m + j])

        cp_wq.start()
        cp_x.start()
        cp_wuk.start()
        for j in range(n_ck):
            cp_ckv(j).start()
        cp_wuv.start()
        cp_w1.start()
        cp_w2.start()
        for j in range(n_m):
            cp_wo_mxu(j).start()
        for j in range(n_v):
            cp_wo_vpu(j).start()
        cp_in(0).start()

        cp_x.wait()
        x = x_v[...].astype(f32)
        mean = jnp.sum(x, axis=1, keepdims=True) * (1.0 / M)
        xc = x - mean
        var = jnp.sum(xc * xc, axis=1, keepdims=True) * (1.0 / M)
        xn = xc * lax.rsqrt(var + _LN_EPS)
        xn_v[...] = jnp.broadcast_to(xn, xn_v.shape).astype(bf16)
        for i in range(M // 128):
            xt_v[i] = jnp.broadcast_to(xn[:, 128 * i:128 * (i + 1)], (H, 128))

        cp_wq.wait()
        cp_in(0).wait()
        cp_fwd(0).start()
        cp_in(1).start()
        head_matvec(xt_v, wq_v, q_v, M // 128)
        qb_v[...] = q_v[...].astype(bf16)

        cp_wuk.wait()
        side_tick(2)

        def qabs_body(i, _):
            lane, row = iotas()
            w = wuk_v[pl.ds(pl.multiple_of(i * 128, 128), 128)].reshape(128 * H, D)
            T = lax.dot_general(qb_v[...], w, (((1,), (1,)), ((), ())),
                                preferred_element_type=f32)
            idx = H * (lane % GRP) + row
            sel = lane // GRP
            out = jnp.zeros((H, 128), f32)
            for t in range(TPB):
                g = jnp.take_along_axis(T[:, 128 * t:128 * (t + 1)], idx, axis=1)
                out = jnp.where(sel == t, g, out)
            qabs_v[i] = (out * (D ** -0.5 * _LOG2E)).astype(bf16)

        lax.fori_loop(0, DC // 128, qabs_body, None)

        def kv_block(b, carry):
            m, l, acc = carry
            qa = jnp.concatenate([qabs_v[i] for i in range(DC // 128)], axis=1)
            c = ckv_v[pl.ds(pl.multiple_of(b * _KV_BLOCK, _KV_BLOCK), _KV_BLOCK), :]
            s = lax.dot_general(qa, c, (((1,), (1,)), ((), ())),
                                preferred_element_type=f32)
            m_new = jnp.maximum(m, jnp.max(s, axis=1, keepdims=True))
            alpha = jnp.exp2(m - m_new)
            p = jnp.exp2(s - m_new)
            l = alpha * l + jnp.sum(p, axis=1, keepdims=True)
            acc = alpha * acc + jnp.dot(p.astype(bf16), c, preferred_element_type=f32)
            return m_new, l, acc

        def kv_chunk(j, carry):
            cp_ckv(j).wait()
            side_tick(3 + j)
            return lax.fori_loop(j * blocks_per_chunk, (j + 1) * blocks_per_chunk,
                                 kv_block, carry)

        _, l, acc = lax.fori_loop(
            0, n_ck, kv_chunk,
            (jnp.full((H, 1), -jnp.inf, f32), jnp.zeros((H, 1), f32), jnp.zeros((H, DC), f32)))
        ctxc = acc / l
        for i in range(DC // 128):
            ctxc_v[i] = ctxc[:, 128 * i:128 * (i + 1)]

        cp_wuv.wait()
        cp_in(n_side - 1).wait()
        cp_fwd(n_side - 2).wait()
        cp_fwd(n_side - 1).start()
        head_matvec(ctxc_v, wuv_v, ctx_v, DC // 128)
        for hh in range(HV):
            r = ctx_v[HM + hh:HM + hh + 1, :]
            cw_v[hh * D:(hh + 1) * D, :] = jnp.broadcast_to(r, (128, D)).T

        cp_w1.wait()
        h1 = lax.dot_general(xn_v[...], w1t_v[...], (((1,), (1,)), ((), ())),
                             preferred_element_type=f32)
        h1_v[...] = (h1 * jax.nn.sigmoid(h1)).astype(bf16)
        cp_w2.wait()
        g = jnp.dot(h1_v[...], w2_v[...], preferred_element_type=f32)[0:1]
        g_v[...] = g * jax.nn.sigmoid(g)

        for j in range(n_m):
            h0, h1_ = h_off[j], h_off[j + 1]
            ctx = ctx_v[...]
            _, row = iotas()
            a = jnp.concatenate(
                [jnp.where(row == h, ctx, 0.0).astype(bf16) for h in range(h0, h1_)], axis=1)
            cp_wo_mxu(j).wait()
            if j == 0:
                cp_fwd(n_side - 1).wait()
            sj = jnp.dot(a, wo_v[h0:h1_].reshape((h1_ - h0) * D, M),
                         preferred_element_type=f32)
            if j > 0:
                sj = sj + s_v[...]
            if j < n_m - 1:
                s_v[...] = sj
            else:
                s = jnp.sum(sj, axis=0, keepdims=True)
                base_v[...] = x_v[...].astype(f32) + s * g_v[...]

        for j in range(n_v):
            h = HM + r_off[j] // D
            r0, R = r_off[j] % D, _WO_VPU_ROWS[j]
            c = cw_v[r_off[j]:r_off[j] + R, :]
            cp_wo_vpu(j).wait()
            w = wo_v[h, r0:r0 + R, :].astype(f32)
            p = w * jnp.concatenate([c] * (M // 128), axis=1)
            acc = jnp.sum(p.reshape(R // 8, 8, M), axis=0)
            if j > 0:
                acc = acc + acc_v[...]
            if j < n_v - 1:
                acc_v[...] = acc
            else:
                s = jnp.sum(acc, axis=0, keepdims=True)
                o_v[...] = (base_v[...] + s * g_v[...]).astype(o_v.dtype)

        cp_out.start()
        cp_out.wait()

    pl.run_scoped(scoped, pltpu.SemaphoreType.DMA((n_sem,)),
                  pltpu.SemaphoreType.DMA((2,)), pltpu.SemaphoreType.DMA((2,)))


@jax.jit
def pallas_recurrent_scan__compressed_kv_cla__dense_activation_silu__decode_kernel(
    A_x: jax.Array,
    A_c_kv: jax.Array,
    A_w_q: jax.Array,
    A_w_uk: jax.Array,
    A_w_uv: jax.Array,
    A_w_o: jax.Array,
    B_x: jax.Array,
    B_w1: jax.Array,
    B_w2: jax.Array,
):
    del B_x
    B, Sq, M = A_x.shape
    _, SK, DC = A_c_kv.shape
    _, H, D = A_w_q.shape
    F = B_w1.shape[1]
    assert B == 1 and Sq == 1, "single-token decode"
    assert D == 128 and 128 % H == 0 and M % 128 == 0 and DC % 128 == 0
    assert SK % (_N_KV_CHUNKS * _KV_BLOCK) == 0
    HM = sum(_WO_MXU_HEADS)
    HV = H - HM
    assert sum(_WO_VPU_ROWS) == HV * D
    assert _WO_SIDE_HEADS < _WO_MXU_HEADS[0]

    def kernel(*refs):
        _kernel_body(H, D, M, DC, SK, HV, *refs)

    hbm = pl.BlockSpec(memory_space=pl.ANY)
    f32, bf16 = jnp.float32, jnp.bfloat16
    return pl.pallas_call(
        kernel,
        in_specs=[hbm] * 8,
        out_specs=hbm,
        out_shape=jax.ShapeDtypeStruct((1, 1, M), A_x.dtype),
        scratch_shapes=[
            pltpu.VMEM((1, M), A_x.dtype),
            pltpu.VMEM((SK, DC), A_c_kv.dtype),
            pltpu.VMEM((M, H, D), A_w_q.dtype),
            pltpu.VMEM((DC, H, D), A_w_uk.dtype),
            pltpu.VMEM((DC, H, D), A_w_uv.dtype),
            pltpu.VMEM((H, D, M), A_w_o.dtype),
            pltpu.VMEM((F, M), B_w1.dtype),
            pltpu.VMEM((F, M), B_w2.dtype),
            pltpu.VMEM((16, M), bf16),
            pltpu.VMEM((M // 128, H, 128), f32),
            pltpu.VMEM((H, D), f32),
            pltpu.VMEM((H, D), bf16),
            pltpu.VMEM((DC // 128, H, 128), bf16),
            pltpu.VMEM((DC // 128, H, 128), f32),
            pltpu.VMEM((H, D), f32),
            pltpu.VMEM((16, F), bf16),
            pltpu.VMEM((1, M), f32),
            pltpu.VMEM((H, M), f32),
            pltpu.VMEM((HV * D, 128), f32),
            pltpu.VMEM((1, M), f32),
            pltpu.VMEM((8, M), f32),
            pltpu.VMEM((1, M), A_x.dtype),
            pltpu.SMEM((2, D, M), A_w_o.dtype),
        ],
        compiler_params=pltpu.CompilerParams(vmem_limit_bytes=64 * 1024 * 1024),
    )(A_x, A_c_kv, A_w_q, A_w_uk, A_w_uv, A_w_o,
      B_w1.T,
      B_w2)
```

```python
import jax
import jax.numpy as jnp
from jax import lax
import jax.experimental.pallas as pl
import jax.experimental.pallas.tpu as pltpu

_LOG2E = 1.4426950408889634
_LN_EPS = 1e-5

_N_KV_CHUNKS = 8
_KV_BLOCK = 1024
_WO_SIDE_HEADS = _N_KV_CHUNKS + 4
_WO_MXU_HEADS = (24, 4, 2)
_WO_VPU_ROWS = (128, 96, 16, 16)


def _kernel_body(H, D, M, DC, SK, HV,
                 x_hbm, ckv_hbm, wq_hbm, wuk_hbm, wuv_hbm, wo_hbm, w1t_hbm, w2_hbm, o_hbm,
                 x_v, ckv_v, wq_v, wuk_v, wuv_v, wo_v, w1t_v, w2_v,
                 xn_v, xt_v, q_v, qb_v, qabs_v, ctxc_v, ctx_v, h1_v, g_v, s_v, cw_v,
                 base_v, acc_v, o_v, sm):
    f32, bf16 = jnp.float32, jnp.bfloat16
    n_ck = _N_KV_CHUNKS
    chunk = SK // n_ck
    blocks_per_chunk = chunk // _KV_BLOCK
    n_m, n_v = len(_WO_MXU_HEADS), len(_WO_VPU_ROWS)
    h_off = [sum(_WO_MXU_HEADS[:j]) for j in range(n_m + 1)]
    r_off = [sum(_WO_VPU_ROWS[:j]) for j in range(n_v + 1)]
    HM = h_off[-1]
    n_sem = 7 + n_ck + n_m + n_v
    n_side = _WO_SIDE_HEADS
    GRP = 128 // H
    TPB = H

    def iotas():
        return (lax.broadcasted_iota(jnp.int32, (H, 128), 1),
                lax.broadcasted_iota(jnp.int32, (H, 128), 0))

    def block_diag(v):
        lane, row = iotas()
        diag = (lane % H) == row
        grp = lane // H
        tiles = []
        for t in range(TPB):
            a = jnp.take_along_axis(v, grp + GRP * t, axis=1)
            tiles.append(jnp.where(diag, a, 0.0).astype(bf16))
        return jnp.concatenate(tiles, axis=1)

    def head_matvec(v_ref, w_ref, out_ref, n_blocks):
        out_ref[...] = jnp.zeros((H, D), f32)

        def body(i, _):
            a = block_diag(v_ref[i])
            w = w_ref[pl.ds(pl.multiple_of(i * 128, 128), 128)].reshape(128 * H, D)
            out_ref[...] += jnp.dot(a, w, preferred_element_type=f32)

        lax.fori_loop(0, n_blocks, body, None)

    def scoped(S, SI, SO):
        cp_wq = pltpu.make_async_copy(wq_hbm, wq_v, S.at[0])
        cp_x = pltpu.make_async_copy(x_hbm.at[0], x_v, S.at[1])
        cp_wuk = pltpu.make_async_copy(wuk_hbm, wuk_v, S.at[2])
        cp_wuv = pltpu.make_async_copy(wuv_hbm, wuv_v, S.at[3])
        cp_w1 = pltpu.make_async_copy(w1t_hbm, w1t_v, S.at[4])
        cp_w2 = pltpu.make_async_copy(w2_hbm, w2_v, S.at[5])
        cp_out = pltpu.make_async_copy(o_v, o_hbm.at[0], S.at[6])

        def cp_ckv(j):
            sl = pl.ds(j * chunk, chunk)
            return pltpu.make_async_copy(ckv_hbm.at[0, sl, :], ckv_v.at[sl, :], S.at[7 + j])

        def cp_wo_mxu(j):
            lo = max(h_off[j], n_side)
            sl = pl.ds(lo, h_off[j + 1] - lo)
            return pltpu.make_async_copy(wo_hbm.at[sl], wo_v.at[sl], S.at[7 + n_ck + j])

        def cp_in(i):
            return pltpu.make_async_copy(wo_hbm.at[i], sm.at[i % 3], SI.at[i % 3])

        def cp_fwd(i):
            return pltpu.make_async_copy(sm.at[i % 3], wo_v.at[i], SO.at[i % 3])

        def side_tick(k):
            cp_in(k).wait()
            cp_fwd(k - 2).wait()
            cp_fwd(k - 1).start()
            cp_in(k + 1).start()

        def cp_wo_vpu(j):
            h = HM + r_off[j] // D
            sl = pl.ds(r_off[j] % D, _WO_VPU_ROWS[j])
            return pltpu.make_async_copy(wo_hbm.at[h, sl, :], wo_v.at[h, sl, :],
                                         S.at[7 + n_ck + n_m + j])

        cp_wq.start()
        cp_x.start()
        cp_wuk.start()
        for j in range(n_ck):
            cp_ckv(j).start()
        cp_wuv.start()
        cp_w1.start()
        cp_w2.start()
        for j in range(n_m):
            cp_wo_mxu(j).start()
        for j in range(n_v):
            cp_wo_vpu(j).start()
        cp_in(0).start()
        cp_in(1).start()

        cp_x.wait()
        x = x_v[...].astype(f32)
        mean = jnp.sum(x, axis=1, keepdims=True) * (1.0 / M)
        xc = x - mean
        var = jnp.sum(xc * xc, axis=1, keepdims=True) * (1.0 / M)
        xn = xc * lax.rsqrt(var + _LN_EPS)
        xn_v[...] = jnp.broadcast_to(xn, xn_v.shape).astype(bf16)
        for i in range(M // 128):
            xt_v[i] = jnp.broadcast_to(xn[:, 128 * i:128 * (i + 1)], (H, 128))

        cp_wq.wait()
        cp_in(0).wait()
        cp_in(1).wait()
        cp_fwd(0).start()
        cp_in(2).start()
        head_matvec(xt_v, wq_v, q_v, M // 128)
        qb_v[...] = q_v[...].astype(bf16)

        cp_wuk.wait()
        side_tick(2)

        def qabs_body(i, _):
            lane, row = iotas()
            w = wuk_v[pl.ds(pl.multiple_of(i * 128, 128), 128)].reshape(128 * H, D)
            T = lax.dot_general(qb_v[...], w, (((1,), (1,)), ((), ())),
                                preferred_element_type=f32)
            idx = H * (lane % GRP) + row
            sel = lane // GRP
            out = jnp.zeros((H, 128), f32)
            for t in range(TPB):
                g = jnp.take_along_axis(T[:, 128 * t:128 * (t + 1)], idx, axis=1)
                out = jnp.where(sel == t, g, out)
            qabs_v[i] = (out * (D ** -0.5 * _LOG2E)).astype(bf16)

        lax.fori_loop(0, DC // 128, qabs_body, None)

        def kv_block(b, carry):
            m, l, acc = carry
            qa = jnp.concatenate([qabs_v[i] for i in range(DC // 128)], axis=1)
            c = ckv_v[pl.ds(pl.multiple_of(b * _KV_BLOCK, _KV_BLOCK), _KV_BLOCK), :]
            s = lax.dot_general(qa, c, (((1,), (1,)), ((), ())),
                                preferred_element_type=f32)
            m_new = jnp.maximum(m, jnp.max(s, axis=1, keepdims=True))
            alpha = jnp.exp2(m - m_new)
            p = jnp.exp2(s - m_new)
            l = alpha * l + jnp.sum(p, axis=1, keepdims=True)
            acc = alpha * acc + jnp.dot(p.astype(bf16), c, preferred_element_type=f32)
            return m_new, l, acc

        def kv_chunk(j, carry):
            cp_ckv(j).wait()
            side_tick(3 + j)
            return lax.fori_loop(j * blocks_per_chunk, (j + 1) * blocks_per_chunk,
                                 kv_block, carry)

        _, l, acc = lax.fori_loop(
            0, n_ck, kv_chunk,
            (jnp.full((H, 1), -jnp.inf, f32), jnp.zeros((H, 1), f32), jnp.zeros((H, DC), f32)))
        ctxc = acc / l
        for i in range(DC // 128):
            ctxc_v[i] = ctxc[:, 128 * i:128 * (i + 1)]

        cp_wuv.wait()
        cp_in(n_side - 1).wait()
        cp_fwd(n_side - 3).wait()
        cp_fwd(n_side - 2).start()
        cp_fwd(n_side - 1).start()
        head_matvec(ctxc_v, wuv_v, ctx_v, DC // 128)
        for hh in range(HV):
            r = ctx_v[HM + hh:HM + hh + 1, :]
            cw_v[hh * D:(hh + 1) * D, :] = jnp.broadcast_to(r, (128, D)).T

        cp_w1.wait()
        h1 = lax.dot_general(xn_v[...], w1t_v[...], (((1,), (1,)), ((), ())),
                             preferred_element_type=f32)
        h1_v[...] = (h1 * jax.nn.sigmoid(h1)).astype(bf16)
        cp_w2.wait()
        g = jnp.dot(h1_v[...], w2_v[...], preferred_element_type=f32)[0:1]
        g_v[...] = g * jax.nn.sigmoid(g)

        n_early = n_side - 2
        segs = [(0, n_early, []),
                (n_side, h_off[1], [cp_wo_mxu(0)]),
                (n_early, n_side, [cp_fwd(n_side - 2), cp_fwd(n_side - 1)])]
        segs += [(h_off[j], h_off[j + 1], [cp_wo_mxu(j)]) for j in range(1, n_m)]
        for k, (h0, h1_, waits) in enumerate(segs):
            ctx = ctx_v[...]
            _, row = iotas()
            a = jnp.concatenate(
                [jnp.where(row == h, ctx, 0.0).astype(bf16) for h in range(h0, h1_)], axis=1)
            for cp in waits:
                cp.wait()
            sj = jnp.dot(a, wo_v[h0:h1_].reshape((h1_ - h0) * D, M),
                         preferred_element_type=f32)
            if k > 0:
                sj = sj + s_v[...]
            if k < len(segs) - 1:
                s_v[...] = sj
            else:
                s = jnp.sum(sj, axis=0, keepdims=True)
                base_v[...] = x_v[...].astype(f32) + s * g_v[...]

        for j in range(n_v):
            h = HM + r_off[j] // D
            r0, R = r_off[j] % D, _WO_VPU_ROWS[j]
            c = cw_v[r_off[j]:r_off[j] + R, :]
            cp_wo_vpu(j).wait()
            w = wo_v[h, r0:r0 + R, :].astype(f32)
            p = w * jnp.concatenate([c] * (M // 128), axis=1)
            acc = jnp.sum(p.reshape(R // 8, 8, M), axis=0)
            if j > 0:
                acc = acc + acc_v[...]
            if j < n_v - 1:
                acc_v[...] = acc
            else:
                s = jnp.sum(acc, axis=0, keepdims=True)
                o_v[...] = (base_v[...] + s * g_v[...]).astype(o_v.dtype)

        cp_out.start()
        cp_out.wait()

    pl.run_scoped(scoped, pltpu.SemaphoreType.DMA((n_sem,)),
                  pltpu.SemaphoreType.DMA((3,)), pltpu.SemaphoreType.DMA((3,)))


@jax.jit
def pallas_recurrent_scan__compressed_kv_cla__dense_activation_silu__decode_kernel(
    A_x: jax.Array,
    A_c_kv: jax.Array,
    A_w_q: jax.Array,
    A_w_uk: jax.Array,
    A_w_uv: jax.Array,
    A_w_o: jax.Array,
    B_x: jax.Array,
    B_w1: jax.Array,
    B_w2: jax.Array,
):
    del B_x
    B, Sq, M = A_x.shape
    _, SK, DC = A_c_kv.shape
    _, H, D = A_w_q.shape
    F = B_w1.shape[1]
    assert B == 1 and Sq == 1, "single-token decode"
    assert D == 128 and 128 % H == 0 and M % 128 == 0 and DC % 128 == 0
    assert SK % (_N_KV_CHUNKS * _KV_BLOCK) == 0
    HM = sum(_WO_MXU_HEADS)
    HV = H - HM
    assert sum(_WO_VPU_ROWS) == HV * D
    assert _WO_SIDE_HEADS < _WO_MXU_HEADS[0]

    def kernel(*refs):
        _kernel_body(H, D, M, DC, SK, HV, *refs)

    hbm = pl.BlockSpec(memory_space=pl.ANY)
    f32, bf16 = jnp.float32, jnp.bfloat16
    return pl.pallas_call(
        kernel,
        in_specs=[hbm] * 8,
        out_specs=hbm,
        out_shape=jax.ShapeDtypeStruct((1, 1, M), A_x.dtype),
        scratch_shapes=[
            pltpu.VMEM((1, M), A_x.dtype),
            pltpu.VMEM((SK, DC), A_c_kv.dtype),
            pltpu.VMEM((M, H, D), A_w_q.dtype),
            pltpu.VMEM((DC, H, D), A_w_uk.dtype),
            pltpu.VMEM((DC, H, D), A_w_uv.dtype),
            pltpu.VMEM((H, D, M), A_w_o.dtype),
            pltpu.VMEM((F, M), B_w1.dtype),
            pltpu.VMEM((F, M), B_w2.dtype),
            pltpu.VMEM((16, M), bf16),
            pltpu.VMEM((M // 128, H, 128), f32),
            pltpu.VMEM((H, D), f32),
            pltpu.VMEM((H, D), bf16),
            pltpu.VMEM((DC // 128, H, 128), bf16),
            pltpu.VMEM((DC // 128, H, 128), f32),
            pltpu.VMEM((H, D), f32),
            pltpu.VMEM((16, F), bf16),
            pltpu.VMEM((1, M), f32),
            pltpu.VMEM((H, M), f32),
            pltpu.VMEM((HV * D, 128), f32),
            pltpu.VMEM((1, M), f32),
            pltpu.VMEM((8, M), f32),
            pltpu.VMEM((1, M), A_x.dtype),
            pltpu.SMEM((3, D, M), A_w_o.dtype),
        ],
        compiler_params=pltpu.CompilerParams(vmem_limit_bytes=64 * 1024 * 1024),
    )(A_x, A_c_kv, A_w_q, A_w_uk, A_w_uv, A_w_o,
      B_w1.T,
      B_w2)
```
